```python
import jax
import jax.numpy as jnp

def _softmax(x, axis=-1):
    return jax.nn.softmax(x, axis=axis)
def _gelu(x):
    return jax.nn.gelu(x, approximate=True)
def _silu(x):
    return jax.nn.silu(x)
def _sigmoid(x):
    return jax.nn.sigmoid(x)
def _layernorm(x, axis=-1, eps=1e-5):
    m = jnp.mean(x, axis=axis, keepdims=True)
    v = jnp.var(x, axis=axis, keepdims=True)
    return (x - m) / jnp.sqrt(v + eps)
def _scatter_add(tgt, idx, src, axis=0):
    return tgt.at[idx].add(src)
def _segment_sum(src, seg, n):
    return jax.ops.segment_sum(src, seg, n)
class _Rng:
    def __init__(self, key):
        self._k = key
    def _next(self):
        self._k, sub = jax.random.split(self._k)
        return sub
    def normal(self, shape):
        return jax.random.normal(self._next(), shape, dtype=jnp.bfloat16)
    def randint(self, lo, hi, shape):
        return jax.random.randint(self._next(), shape, lo, hi, dtype=jnp.int32)
    def uniform(self, shape, lo=0.0, hi=1.0):
        return jax.random.uniform(self._next(), shape, jnp.bfloat16, lo, hi)
    def permutation(self, n):
        return jax.random.permutation(self._next(), n)


kernel_name = 'sequential_preLN__sliding_block_cached__mixer_s_mlp__decode'

def setup_inputs():
    _rng = _Rng(jax.random.key(int.from_bytes(__import__("os").urandom(4), "little")))
    _w = (lambda a: (lambda t: t.astype(jnp.bfloat16) if jnp.issubdtype(t.dtype, jnp.floating) else t)(jnp.asarray(a)))
    def _A_setup():
        B, Sq, D = 1, 1, 640
        Hq, Hkv, Sk, Dh = 32, 32, 32768, 192
        assert Hq % Hkv == 0, (Hq, Hkv)
        return {
            "x": _w((lambda *s: _rng.normal(s) * 0.05)(B, Sq, D)),
            "k_cache": _w((lambda *s: _rng.normal(s) * 0.05)(B, Hkv, Sk, Dh)),
            "v_cache": _w((lambda *s: _rng.normal(s) * 0.05)(B, Hkv, Sk, Dh)),
            "wq": _w((lambda *s: _rng.normal(s) * 0.05)(D, Hq * Dh) * (D ** -0.5)),
            "wo": _w((lambda *s: _rng.normal(s) * 0.05)(Hq * Dh, D) * ((Hq * Dh) ** -0.5)),
        }
    _A_in = _A_setup()

    def _B_setup():
        B, S, D, F = 1, 1, 640, 1536
        return {
            "x":  _w((lambda *s: _rng.normal(s) * 0.05)(B, S, D)),
            "w1": _w((lambda *s: _rng.normal(s) * 0.05)(D, D) * (D ** -0.5)),
            "w2": _w((lambda *s: _rng.normal(s) * 0.05)(D, D) * (D ** -0.5)),
            "w3": _w((lambda *s: _rng.normal(s) * 0.05)(D, F) * (D ** -0.5)),
            "w4": _w((lambda *s: _rng.normal(s) * 0.05)(F, D) * (F ** -0.5)),
        }
    _B_in = _B_setup()

    return {
        "A_x": _A_in["x"],
        "A_k_cache": _A_in["k_cache"],
        "A_v_cache": _A_in["v_cache"],
        "A_wq": _A_in["wq"],
        "A_wo": _A_in["wo"],
        "B_x": _B_in["x"],
        "B_w1": _B_in["w1"],
        "B_w2": _B_in["w2"],
        "B_w3": _B_in["w3"],
        "B_w4": _B_in["w4"],
    }

def reference(A_x, A_k_cache, A_v_cache, A_wq, A_wo, B_x, B_w1, B_w2, B_w3, B_w4):
    def _A_ref(x, k_cache, v_cache, wq, wo):
        B, Sq, D = x.shape
        Hq, Dh = 32, 192
        Hkv, Sk = k_cache.shape[1], k_cache.shape[2]
        W = min(4096, max(256, Sk // 4))
        rep = Hq // Hkv
        q = (lambda x, *d: x.transpose(*d))((x @ wq).reshape(B, Sq, Hq, Dh), 0, 2, 1, 3)
        k = jnp.repeat(k_cache[:, :, Sk - W:, :], rep, axis=1)
        v = jnp.repeat(v_cache[:, :, Sk - W:, :], rep, axis=1)
        scores = jnp.einsum("bhqd,bhkd->bhqk", q, k) * (Dh ** -0.5)
        p = _softmax(scores, axis=-1)
        o = jnp.einsum("bhqk,bhkd->bhqd", p, v)
        return (lambda x, *d: x.transpose(*d))(o, 0, 2, 1, 3).reshape(B, Sq, Hq * Dh) @ wo

    def _B_ref(x, w1, w2, w3, w4):
        B, S, D = x.shape
        h = _gelu(_layernorm(x, axis=-1) @ w1)
        c = D // 4
        g0 = jnp.pad(h[:, :, 0*c:1*c], ((0, 0), (1, 0), (0, 0)))[:, :S, :]
        g1 = jnp.pad(h[:, :, 1*c:2*c], ((0, 0), (0, 1), (0, 0)))[:, 1:, :]
        g2 = jnp.pad(h[:, :, 2*c:3*c], ((0, 0), (2, 0), (0, 0)))[:, :S, :]
        g3 = jnp.pad(h[:, :, 3*c:   ], ((0, 0), (0, 2), (0, 0)))[:, 2:, :]
        hs = jnp.concatenate([g0, g1, g2, g3], axis=-1) @ w2
        x1 = x + hs
        h2 = _gelu(_layernorm(x1, axis=-1) @ w3) @ w4
        return x1 + h2

    x = A_x
    h = x + _A_ref(_layernorm(x, axis=-1), A_k_cache, A_v_cache, A_wq, A_wo)
    h2 = h + _B_ref(_layernorm(h, axis=-1), B_w1, B_w2, B_w3, B_w4)
    return h2
```

```python
import jax
import jax.numpy as jnp
from jax import lax
import jax.experimental.pallas as pl
import jax.experimental.pallas.tpu as pltpu

_EPS = 1e-5
_LOOK = 2
_CR, _CC = 8, 2048
_WO_ROWS = 16
_W4_GROUPS = 4


def _layernorm(x):
    m = jnp.mean(x, axis=-1, keepdims=True)
    d = x - m
    v = jnp.mean(d * d, axis=-1, keepdims=True)
    return d / jnp.sqrt(v + _EPS)


@jax.jit
def pallas_sequential_preLN__sliding_block_cached__mixer_s_mlp__decode_kernel(
    A_x: jax.Array,
    A_k_cache: jax.Array,
    A_v_cache: jax.Array,
    A_wq: jax.Array,
    A_wo: jax.Array,
    B_x: jax.Array,
    B_w1: jax.Array,
    B_w2: jax.Array,
    B_w3: jax.Array,
    B_w4: jax.Array,
):
    del B_x, B_w1, B_w2
    B, Sq, D = A_x.shape
    _, H, SK, DH = A_k_cache.shape
    F = B_w3.shape[1]
    HD = H * DH
    assert (B, Sq) == (1, 1) and A_wq.shape == (D, HD) and A_wo.shape == (HD, D)
    W = min(4096, max(256, SK // 4))
    K0 = SK - W
    NS = _LOOK + 1
    scale = DH ** -0.5
    kv_pieces = [(r, c) for r in range(0, DH, _CR) for c in range(0, W, _CC)]
    g_rows = F // _W4_GROUPS

    def kernel(x_hbm, kt_hbm, vt_hbm, wq_hbm, wo_hbm, w3_hbm, w4_hbm, out_ref,
               x_v, wq_v, wo_v, w3_v, w4_v, k_buf, v_buf, q_v,
               sem_k, sem_v, sem_w):
        def start_pair(h):
            slot = h % NS
            for (r, c) in kv_pieces:
                pltpu.make_async_copy(kt_hbm.at[0, h, pl.ds(r, _CR), pl.ds(K0 + c, _CC)],
                                      k_buf.at[slot, pl.ds(r, _CR), pl.ds(c, _CC)],
                                      sem_k.at[slot]).start(priority=0)
                pltpu.make_async_copy(vt_hbm.at[0, h, pl.ds(r, _CR), pl.ds(K0 + c, _CC)],
                                      v_buf.at[slot, pl.ds(r, _CR), pl.ds(c, _CC)],
                                      sem_v.at[slot]).start(priority=1)

        def wait_pair(h):
            slot = h % NS
            pltpu.make_async_copy(k_buf.at[slot], k_buf.at[slot], sem_k.at[slot]).wait()
            pltpu.make_async_copy(v_buf.at[slot], v_buf.at[slot], sem_v.at[slot]).wait()

        def start_wq():
            def body(i, carry):
                r = pl.multiple_of(i * 16, 16)
                n = 0
                for rr in (0, 8):
                    for c in range(0, HD, _CC):
                        pltpu.make_async_copy(wq_hbm.at[pl.ds(r + rr, 8), pl.ds(c, _CC)],
                                              wq_v.at[pl.ds(r + rr, 8), pl.ds(c, _CC)],
                                              sem_w.at[0]).start(priority=n % 2)
                        n += 1
                return carry
            lax.fori_loop(0, D // 16, body, 0)

        def start_rows(src, dst, row0, nrows, step, sem):
            def body(i, carry):
                for j in range(2):
                    r = pl.multiple_of(row0 + (2 * i + j) * step, 8)
                    pltpu.make_async_copy(src.at[pl.ds(r, step)], dst.at[pl.ds(r, step)],
                                          sem).start(priority=j)
                return carry
            lax.fori_loop(0, nrows // (2 * step), body, 0)

        copy_x = pltpu.make_async_copy(x_hbm, x_v, sem_w.at[1])
        copy_x.start()
        start_wq()
        start_pair(0)
        start_rows(wo_hbm, wo_v, 0, HD, _WO_ROWS, sem_w.at[2])
        for h in range(1, _LOOK):
            start_pair(h)

        copy_x.wait()
        x = x_v[0].astype(jnp.float32)
        xn = jnp.broadcast_to(_layernorm(x), (8, D)).astype(jnp.bfloat16)
        pltpu.make_async_copy(wq_v, wq_v, sem_w.at[0]).wait()
        q = jnp.dot(xn, wq_v[...], preferred_element_type=jnp.float32)
        for h in range(H):
            q_v[h] = q[:, h * DH:(h + 1) * DH]
        pltpu.make_async_copy(wo_v, wo_v, sem_w.at[2]).wait()

        def head(h, attn):
            slot = h % NS
            qh = q_v[h].astype(jnp.bfloat16)
            s = jnp.dot(qh, k_buf[slot], preferred_element_type=jnp.float32) * scale
            m = jnp.max(s, axis=-1, keepdims=True)
            e = jnp.exp(s - m)
            l = jnp.sum(e, axis=-1, keepdims=True)
            o = lax.dot_general(e.astype(jnp.bfloat16), v_buf[slot], (((1,), (1,)), ((), ())),
                                preferred_element_type=jnp.float32)
            o = (o / l).astype(jnp.bfloat16)
            r0 = pl.multiple_of(h * DH, DH)
            return attn + jnp.dot(o, wo_v[pl.ds(r0, DH), :], preferred_element_type=jnp.float32)

        def loop_body(h, attn):
            wait_pair(h)
            attn = head(h, attn)
            start_pair(h + _LOOK)
            return attn

        attn = lax.fori_loop(0, H - _LOOK, loop_body, jnp.zeros((8, D), jnp.float32))

        def start_w3():
            def body(i, carry):
                for j in range(2):
                    r = pl.multiple_of((2 * i + j) * 8, 8)
                    pltpu.make_async_copy(w3_hbm.at[pl.ds(r, 8)], w3_v.at[pl.ds(r, 8)],
                                          sem_w.at[1]).start(priority=j)
                return carry
            lax.fori_loop(0, D // 16, body, 0)

        def start_w4():
            for g in range(_W4_GROUPS):
                start_rows(w4_hbm, w4_v, g * g_rows, g_rows, _WO_ROWS, sem_w.at[3 + g])

        tail = [start_w3, start_w4]
        for t, h in enumerate(range(H - _LOOK, H)):
            wait_pair(h)
            if t < len(tail):
                tail[t]()
            attn = head(h, attn)
        for t in range(_LOOK, len(tail)):
            tail[t]()

        hres = x + attn
        y = _layernorm(hres)
        z = _layernorm(y).astype(jnp.bfloat16)
        pltpu.make_async_copy(w3_v, w3_v, sem_w.at[1]).wait()
        u = jnp.dot(z, w3_v[...], preferred_element_type=jnp.float32)
        u = jax.nn.gelu(u, approximate=True).astype(jnp.bfloat16)
        acc = hres + y
        for g in range(_W4_GROUPS):
            rows = w4_v.at[pl.ds(g * g_rows, g_rows)]
            pltpu.make_async_copy(rows, rows, sem_w.at[3 + g]).wait()
            acc = acc + jnp.dot(u[:, g * g_rows:(g + 1) * g_rows],
                                w4_v[g * g_rows:(g + 1) * g_rows, :],
                                preferred_element_type=jnp.float32)
        out_ref[0] = acc[0:1].astype(out_ref.dtype)

    any_spec = pl.BlockSpec(memory_space=pl.ANY)
    bf = jnp.bfloat16
    return pl.pallas_call(
        kernel,
        out_shape=jax.ShapeDtypeStruct((B, Sq, D), A_x.dtype),
        in_specs=[any_spec] * 7,
        out_specs=pl.BlockSpec(memory_space=pltpu.VMEM),
        scratch_shapes=[
            pltpu.VMEM((B, Sq, D), bf),
            pltpu.VMEM((D, HD), bf), pltpu.VMEM((HD, D), bf),
            pltpu.VMEM((D, F), bf), pltpu.VMEM((F, D), bf),
            pltpu.VMEM((NS, DH, W), bf), pltpu.VMEM((NS, DH, W), bf),
            pltpu.VMEM((H, 8, DH), jnp.float32),
            pltpu.SemaphoreType.DMA((NS,)), pltpu.SemaphoreType.DMA((NS,)),
            pltpu.SemaphoreType.DMA((3 + _W4_GROUPS,)),
        ],
        compiler_params=pltpu.CompilerParams(vmem_limit_bytes=64 * 1024 * 1024),
    )(A_x, jnp.swapaxes(A_k_cache, 2, 3), jnp.swapaxes(A_v_cache, 2, 3),
      A_wq, A_wo, B_w3, B_w4)
```

```python
import jax
import jax.numpy as jnp
from jax import lax
import jax.experimental.pallas as pl
import jax.experimental.pallas.tpu as pltpu

_EPS = 1e-5
_LOOK = 2
_KR, _KC = 32, 512
_NB = 4
_WO_ROWS = 32
_W3_ROWS = 8
_W4_ROWS = 16
_W4_GROUPS = 4
_QJ = 384


def _layernorm(x):
    m = jnp.mean(x, axis=-1, keepdims=True)
    d = x - m
    v = jnp.mean(d * d, axis=-1, keepdims=True)
    return d / jnp.sqrt(v + _EPS)


def _loop(n, body):
    def step(i, carry):
        body(i)
        return carry
    lax.fori_loop(0, n, step, 0)


@jax.jit
def pallas_sequential_preLN__sliding_block_cached__mixer_s_mlp__decode_kernel(
    A_x: jax.Array,
    A_k_cache: jax.Array,
    A_v_cache: jax.Array,
    A_wq: jax.Array,
    A_wo: jax.Array,
    B_x: jax.Array,
    B_w1: jax.Array,
    B_w2: jax.Array,
    B_w3: jax.Array,
    B_w4: jax.Array,
):
    del B_x, B_w1, B_w2
    B, Sq, D = A_x.shape
    _, H, SK, DH = A_k_cache.shape
    F = B_w3.shape[1]
    HD = H * DH
    assert (B, Sq) == (1, 1) and A_wq.shape == (D, HD) and A_wo.shape == (HD, D)
    W = min(4096, max(256, SK // 4))
    K0 = SK - W
    NS = _LOOK + 1
    scale = DH ** -0.5
    CB = W // _NB
    NRP = DH // _KR
    NG = 2 * _NB
    PPG = NRP * (W // _KC) // NG
    g_rows = F // _W4_GROUPS
    assert W % CB == 0 and DH % _KR == 0 and W % _KC == 0 and PPG * NG == NRP * (W // _KC)

    def kernel(x_hbm, kt_hbm, vt_hbm, wq_hbm, wo_hbm, w3_hbm, w4_hbm, out_ref,
               x_v, wq_v, wo_v, w3_v, w4_v, k_buf, v_buf, q_v, s_v,
               sem_k, sem_v, sem_w):

        def start_kv_group(h, g):
            slot = h % NS
            for t in range(PPG):
                n = g * PPG + t
                c = pl.multiple_of((n // NRP) * _KC, _KC)
                r = pl.multiple_of((n % NRP) * _KR, _KR)
                pltpu.make_async_copy(kt_hbm.at[0, h, pl.ds(r, _KR), pl.ds(K0 + c, _KC)],
                                      k_buf.at[slot, pl.ds(r, _KR), pl.ds(c, _KC)],
                                      sem_k.at[slot]).start(priority=0)
                pltpu.make_async_copy(vt_hbm.at[0, h, pl.ds(r, _KR), pl.ds(K0 + c, _KC)],
                                      v_buf.at[slot, pl.ds(r, _KR), pl.ds(c, _KC)],
                                      sem_v.at[slot]).start(priority=1)

        def start_kv(h):
            _loop(NG, lambda g: start_kv_group(h, g))

        def wait_kv(h):
            slot = h % NS
            pltpu.make_async_copy(k_buf.at[slot], k_buf.at[slot], sem_k.at[slot]).wait()
            pltpu.make_async_copy(v_buf.at[slot], v_buf.at[slot], sem_v.at[slot]).wait()

        def start_wq():
            def col_block(i):
                c = pl.multiple_of(i * _KC, _KC)

                def row_pair(j):
                    for t in range(2):
                        r = pl.multiple_of((2 * j + t) * _KR, _KR)
                        pltpu.make_async_copy(wq_hbm.at[pl.ds(r, _KR), pl.ds(c, _KC)],
                                              wq_v.at[pl.ds(r, _KR), pl.ds(c, _KC)],
                                              sem_w.at[0]).start(priority=t)
                _loop(D // _KR // 2, row_pair)
            _loop(HD // _KC, col_block)

        def start_row_pairs(src, dst, step, sem, base, half, i0, n):
            for t in range(n):
                for j in range(2):
                    r = pl.multiple_of(base + j * half + (i0 + t) * step, step)
                    pltpu.make_async_copy(src.at[pl.ds(r, step)], dst.at[pl.ds(r, step)],
                                          sem).start(priority=j)

        copy_x = pltpu.make_async_copy(x_hbm, x_v, sem_w.at[1])
        copy_x.start()
        start_wq()
        start_kv(0)
        copy_x.wait()
        x = x_v[0].astype(jnp.float32)
        xn = jnp.broadcast_to(_layernorm(x), (8, D)).astype(jnp.bfloat16)
        pltpu.make_async_copy(wq_v, wq_v, sem_w.at[0]).wait()

        heads_per_slice = _QJ // DH
        n_q = HD // _QJ
        wo_pairs = HD // (2 * _WO_ROWS) // n_q

        def q_slice(j):
            c = pl.multiple_of(j * _QJ, _QJ)
            q = jnp.dot(xn, wq_v[:, pl.ds(c, _QJ)], preferred_element_type=jnp.float32)
            for t in range(heads_per_slice):
                q_v[j * heads_per_slice + t] = q[:, t * DH:(t + 1) * DH]
            start_row_pairs(wo_hbm, wo_v, _WO_ROWS, sem_w.at[2], 0, HD // 2, j * wo_pairs, wo_pairs)
        _loop(n_q, q_slice)
        start_kv(1)
        pltpu.make_async_copy(wo_v, wo_v, sem_w.at[2]).wait()

        w3_pairs = D // (2 * _W3_ROWS) // _NB
        w4_slices = _NB // _W4_GROUPS
        w4_pairs = g_rows // (2 * _W4_ROWS) // w4_slices

        def issue(h, c, phase):
            @pl.when(h + _LOOK < H)
            def _():
                start_kv_group(h + _LOOK, phase * _NB + c)
            if phase == 0:
                @pl.when(h + _LOOK == H)
                def _():
                    start_row_pairs(w3_hbm, w3_v, _W3_ROWS, sem_w.at[1], 0, D // 2,
                                    c * w3_pairs, w3_pairs)

                @pl.when(h + _LOOK == H + 1)
                def _():
                    g = c // w4_slices
                    start_row_pairs(w4_hbm, w4_v, _W4_ROWS, sem_w.at[3 + g], g * g_rows,
                                    g_rows // 2, (c % w4_slices) * w4_pairs, w4_pairs)

        def head(h, attn):
            wait_kv(h)
            slot = h % NS
            qh = q_v[h].astype(jnp.bfloat16)

            def qk_slice(c, m):
                c0 = pl.multiple_of(c * CB, CB)
                s = jnp.dot(qh, k_buf[slot, :, pl.ds(c0, CB)],
                            preferred_element_type=jnp.float32) * scale
                s_v[:, pl.ds(c0, CB)] = s
                for t in range(CB // 128):
                    m = jnp.maximum(m, s[:, t * 128:(t + 1) * 128])
                issue(h, c, 0)
                return m
            m = lax.fori_loop(0, _NB, qk_slice, jnp.full((8, 128), -jnp.inf, jnp.float32))
            m = jnp.max(m, axis=-1, keepdims=True)

            def pv_slice(c, carry):
                o, l = carry
                c0 = pl.multiple_of(c * CB, CB)
                e = jnp.exp(s_v[:, pl.ds(c0, CB)] - m)
                for t in range(CB // 128):
                    l = l + e[:, t * 128:(t + 1) * 128]
                o = o + lax.dot_general(e.astype(jnp.bfloat16), v_buf[slot, :, pl.ds(c0, CB)],
                                        (((1,), (1,)), ((), ())),
                                        preferred_element_type=jnp.float32)
                issue(h, c, 1)
                return o, l
            o, l = lax.fori_loop(0, _NB, pv_slice, (jnp.zeros((8, DH), jnp.float32),
                                                    jnp.zeros((8, 128), jnp.float32)))
            o = (o / jnp.sum(l, axis=-1, keepdims=True)).astype(jnp.bfloat16)
            r0 = pl.multiple_of(h * DH, DH)
            return attn + jnp.dot(o, wo_v[pl.ds(r0, DH), :], preferred_element_type=jnp.float32)

        attn = lax.fori_loop(0, H, head, jnp.zeros((8, D), jnp.float32))

        hres = x + attn
        y = _layernorm(hres)
        z = _layernorm(y).astype(jnp.bfloat16)
        pltpu.make_async_copy(w3_v, w3_v, sem_w.at[1]).wait()
        u = jnp.dot(z, w3_v[...], preferred_element_type=jnp.float32)
        u = jax.nn.gelu(u, approximate=True).astype(jnp.bfloat16)
        acc = hres + y
        for g in range(_W4_GROUPS):
            rows = w4_v.at[pl.ds(g * g_rows, g_rows)]
            pltpu.make_async_copy(rows, rows, sem_w.at[3 + g]).wait()
            acc = acc + jnp.dot(u[:, g * g_rows:(g + 1) * g_rows],
                                w4_v[g * g_rows:(g + 1) * g_rows, :],
                                preferred_element_type=jnp.float32)
        out_ref[0] = acc[0:1].astype(out_ref.dtype)

    any_spec = pl.BlockSpec(memory_space=pl.ANY)
    bf = jnp.bfloat16
    return pl.pallas_call(
        kernel,
        out_shape=jax.ShapeDtypeStruct((B, Sq, D), A_x.dtype),
        in_specs=[any_spec] * 7,
        out_specs=pl.BlockSpec(memory_space=pltpu.VMEM),
        scratch_shapes=[
            pltpu.VMEM((B, Sq, D), bf),
            pltpu.VMEM((D, HD), bf), pltpu.VMEM((HD, D), bf),
            pltpu.VMEM((D, F), bf), pltpu.VMEM((F, D), bf),
            pltpu.VMEM((NS, DH, W), bf), pltpu.VMEM((NS, DH, W), bf),
            pltpu.VMEM((H, 8, DH), jnp.float32),
            pltpu.VMEM((8, W), jnp.float32),
            pltpu.SemaphoreType.DMA((NS,)), pltpu.SemaphoreType.DMA((NS,)),
            pltpu.SemaphoreType.DMA((3 + _W4_GROUPS,)),
        ],
        compiler_params=pltpu.CompilerParams(vmem_limit_bytes=64 * 1024 * 1024),
    )(A_x, jnp.swapaxes(A_k_cache, 2, 3), jnp.swapaxes(A_v_cache, 2, 3),
      A_wq, A_wo, B_w3, B_w4)
```

```python
import jax
import jax.numpy as jnp
from jax import lax
import jax.experimental.pallas as pl
import jax.experimental.pallas.tpu as pltpu

_EPS = 1e-5
_LOOK = 2
_SLOTS = 4
_KR, _KC = 32, 512
_NB = 4
_WQ_ROWS, _WQ_COLS = 8, 2048
_WO_ROWS = 16
_W3_ROWS = 8
_W4_ROWS = 32
_QJ = 384


def _layernorm(x):
    m = jnp.mean(x, axis=-1, keepdims=True)
    d = x - m
    v = jnp.mean(d * d, axis=-1, keepdims=True)
    return d / jnp.sqrt(v + _EPS)


def _loop(n, body):
    def step(i, carry):
        body(i)
        return carry
    lax.fori_loop(0, n, step, 0)


@jax.jit
def pallas_sequential_preLN__sliding_block_cached__mixer_s_mlp__decode_kernel(
    A_x: jax.Array,
    A_k_cache: jax.Array,
    A_v_cache: jax.Array,
    A_wq: jax.Array,
    A_wo: jax.Array,
    B_x: jax.Array,
    B_w1: jax.Array,
    B_w2: jax.Array,
    B_w3: jax.Array,
    B_w4: jax.Array,
):
    del B_x, B_w1, B_w2
    B, Sq, D = A_x.shape
    _, H, SK, DH = A_k_cache.shape
    F = B_w3.shape[1]
    HD = H * DH
    assert (B, Sq) == (1, 1) and A_wq.shape == (D, HD) and A_wo.shape == (HD, D)
    W = min(4096, max(256, SK // 4))
    K0 = SK - W
    scale = DH ** -0.5
    CB = W // _NB
    NG = W // _KC
    n_w3 = D // (2 * _W3_ROWS) // _NB
    w4_rows = F // _NB
    n_w4 = w4_rows // (2 * _W4_ROWS)
    assert NG == 2 * _NB and DH % _KR == 0 and _NB <= _SLOTS
    assert (D // 2) % _WQ_ROWS == 0 and HD % _WQ_COLS == 0 and HD % _QJ == 0 and _QJ % DH == 0
    assert n_w3 * _NB * 2 * _W3_ROWS == D and n_w4 * 2 * _W4_ROWS == w4_rows

    def kernel(x_hbm, kt_hbm, vt_hbm, wq_hbm, wo_hbm, w3_hbm, w4_hbm, out_ref,
               x_v, wq_v, wo_v, w3_v, w4_v, k_buf, v_buf, q_v, s_v,
               sem_k, sem_v, sem_w):

        def start_kv_group(h, g):
            slot = h & (_SLOTS - 1)
            c = pl.multiple_of(g * _KC, _KC)
            for r in range(0, DH, _KR):
                pltpu.make_async_copy(kt_hbm.at[0, h, pl.ds(r, _KR), pl.ds(K0 + c, _KC)],
                                      k_buf.at[slot, pl.ds(r, _KR), pl.ds(c, _KC)],
                                      sem_k.at[slot]).start(priority=0)
                pltpu.make_async_copy(vt_hbm.at[0, h, pl.ds(r, _KR), pl.ds(K0 + c, _KC)],
                                      v_buf.at[slot, pl.ds(r, _KR), pl.ds(c, _KC)],
                                      sem_v.at[slot]).start(priority=1)

        def wait_kv(h):
            slot = h & (_SLOTS - 1)
            pltpu.make_async_copy(k_buf.at[slot], k_buf.at[slot], sem_k.at[slot]).wait()
            pltpu.make_async_copy(v_buf.at[slot], v_buf.at[slot], sem_v.at[slot]).wait()

        def start_row_pairs(src, dst, sem, step, base, half, i0, n, cols=None):
            for t in range(n):
                for c in (range(0, src.shape[1], cols) if cols else (None,)):
                    for j in range(2):
                        r = pl.multiple_of(base + j * half + (i0 + t) * step, step)
                        idx = (pl.ds(r, step),) if c is None else (pl.ds(r, step), pl.ds(c, cols))
                        pltpu.make_async_copy(src.at[idx], dst.at[idx], sem).start(priority=j)

        def wait_all(buf, sem):
            pltpu.make_async_copy(buf, buf, sem).wait()

        copy_x = pltpu.make_async_copy(x_hbm, x_v, sem_w.at[0])
        copy_x.start()
        _loop(D // 2 // _WQ_ROWS,
              lambda i: start_row_pairs(wq_hbm, wq_v, sem_w.at[1], _WQ_ROWS, 0, D // 2, i, 1, _WQ_COLS))
        _loop(NG, lambda g: start_kv_group(0, g))
        copy_x.wait()
        x = x_v[0].astype(jnp.float32)
        xn = jnp.broadcast_to(_layernorm(x), (8, D)).astype(jnp.bfloat16)
        wait_all(wq_v, sem_w.at[1])

        heads_per_slice = _QJ // DH
        n_q = HD // _QJ
        n_wo = HD // (2 * _WO_ROWS) // n_q

        def q_slice(j):
            c = pl.multiple_of(j * _QJ, _QJ)
            q = jnp.dot(xn, wq_v[:, pl.ds(c, _QJ)], preferred_element_type=jnp.float32)
            for t in range(heads_per_slice):
                q_v[j * heads_per_slice + t] = q[:, t * DH:(t + 1) * DH]
            start_row_pairs(wo_hbm, wo_v, sem_w.at[0], _WO_ROWS, 0, HD // 2, j * n_wo, n_wo)
        _loop(n_q, q_slice)
        _loop(NG, lambda g: start_kv_group(1, g))
        wait_all(wo_v, sem_w.at[0])

        def head(h, attn, issue_qk, issue_pv):
            wait_kv(h)
            slot = h & (_SLOTS - 1)
            qh = q_v[h].astype(jnp.bfloat16)

            def qk_slice(c, m):
                c0 = pl.multiple_of(c * CB, CB)
                s = jnp.dot(qh, k_buf[slot, :, pl.ds(c0, CB)],
                            preferred_element_type=jnp.float32) * scale
                s_v[:, pl.ds(c0, CB)] = s
                for t in range(CB // 128):
                    m = jnp.maximum(m, s[:, t * 128:(t + 1) * 128])
                issue_qk(c)
                return m
            m = lax.fori_loop(0, _NB, qk_slice, jnp.full((8, 128), -jnp.inf, jnp.float32))
            m = jnp.max(m, axis=-1, keepdims=True)

            def pv_slice(c, carry):
                o, l = carry
                c0 = pl.multiple_of(c * CB, CB)
                e = jnp.exp(s_v[:, pl.ds(c0, CB)] - m)
                for t in range(CB // 128):
                    l = l + e[:, t * 128:(t + 1) * 128]
                o = o + lax.dot_general(e.astype(jnp.bfloat16), v_buf[slot, :, pl.ds(c0, CB)],
                                        (((1,), (1,)), ((), ())),
                                        preferred_element_type=jnp.float32)
                issue_pv(c)
                return o, l
            o, l = lax.fori_loop(0, _NB, pv_slice, (jnp.zeros((8, DH), jnp.float32),
                                                    jnp.zeros((8, 128), jnp.float32)))
            o = (o / jnp.sum(l, axis=-1, keepdims=True)).astype(jnp.bfloat16)
            r0 = pl.multiple_of(h * DH, DH)
            return attn + jnp.dot(o, wo_v[pl.ds(r0, DH), :], preferred_element_type=jnp.float32)

        attn = lax.fori_loop(
            0, H - _LOOK,
            lambda h, a: head(h, a,
                              lambda c: start_kv_group(h + _LOOK, c),
                              lambda c: start_kv_group(h + _LOOK, _NB + c)),
            jnp.zeros((8, D), jnp.float32))

        def nothing(c):
            del c
        attn = head(H - 2, attn,
                    lambda c: start_row_pairs(w3_hbm, w3_v, sem_w.at[1], _W3_ROWS, 0, D // 2,
                                              c * n_w3, n_w3),
                    nothing)
        attn = head(H - 1, attn,
                    lambda c: start_row_pairs(w4_hbm, w4_v, sem_k.at[c], _W4_ROWS, c * w4_rows,
                                              w4_rows // 2, 0, n_w4),
                    nothing)

        hres = x + attn
        y = _layernorm(hres)
        z = _layernorm(y).astype(jnp.bfloat16)
        wait_all(w3_v, sem_w.at[1])
        u = jnp.dot(z, w3_v[...], preferred_element_type=jnp.float32)
        u = jax.nn.gelu(u, approximate=True).astype(jnp.bfloat16)
        acc = hres + y
        for g in range(_NB):
            lo, hi = g * w4_rows, (g + 1) * w4_rows
            wait_all(w4_v.at[pl.ds(lo, w4_rows)], sem_k.at[g])
            acc = acc + jnp.dot(u[:, lo:hi], w4_v[lo:hi, :], preferred_element_type=jnp.float32)
        out_ref[0] = acc[0:1].astype(out_ref.dtype)

    any_spec = pl.BlockSpec(memory_space=pl.ANY)
    bf = jnp.bfloat16
    return pl.pallas_call(
        kernel,
        out_shape=jax.ShapeDtypeStruct((B, Sq, D), A_x.dtype),
        in_specs=[any_spec] * 7,
        out_specs=pl.BlockSpec(memory_space=pltpu.VMEM),
        scratch_shapes=[
            pltpu.VMEM((B, Sq, D), bf),
            pltpu.VMEM((D, HD), bf), pltpu.VMEM((HD, D), bf),
            pltpu.VMEM((D, F), bf), pltpu.VMEM((F, D), bf),
            pltpu.VMEM((_SLOTS, DH, W), bf), pltpu.VMEM((_SLOTS, DH, W), bf),
            pltpu.VMEM((H, 8, DH), jnp.float32),
            pltpu.VMEM((8, W), jnp.float32),
            pltpu.SemaphoreType.DMA((_SLOTS,)), pltpu.SemaphoreType.DMA((_SLOTS,)),
            pltpu.SemaphoreType.DMA((2,)),
        ],
        compiler_params=pltpu.CompilerParams(vmem_limit_bytes=64 * 1024 * 1024),
    )(A_x, jnp.swapaxes(A_k_cache, 2, 3), jnp.swapaxes(A_v_cache, 2, 3),
      A_wq, A_wo, B_w3, B_w4)
```
